```python
import os as _os
_os.environ.setdefault('JAX_PLATFORMS', 'cpu')
import jax
import jax.numpy as jnp

def _softmax(x, axis=-1):
    return jax.nn.softmax(x, axis=axis)

def _gelu(x):
    return jax.nn.gelu(x, approximate=True)

def _silu(x):
    return jax.nn.silu(x)

def _sigmoid(x):
    return jax.nn.sigmoid(x)

def _layernorm(x, axis=-1, eps=1e-05):
    m = jnp.mean(x, axis=axis, keepdims=True)
    v = jnp.var(x, axis=axis, keepdims=True)
    return (x - m) / jnp.sqrt(v + eps)

def _scatter_add(tgt, idx, src, axis=0):
    return tgt.at[idx].add(src)

def _segment_sum(src, seg, n):
    return jax.ops.segment_sum(src, seg, n)

class _Rng:

    def __init__(self, key):
        self._k = key

    def _next(self):
        self._k, sub = jax.random.split(self._k)
        return sub

    def normal(self, shape):
        return jax.random.normal(self._next(), shape, dtype=jnp.bfloat16)

    def randint(self, lo, hi, shape):
        return jax.random.randint(self._next(), shape, lo, hi, dtype=jnp.int32)

    def uniform(self, shape, lo=0.0, hi=1.0):
        return jax.random.uniform(self._next(), shape, jnp.bfloat16, lo, hi)

    def permutation(self, n):
        return jax.random.permutation(self._next(), n)
kernel_name = 'adaLN_cond__sliding_local_dilated__dense_activation_relu__prompt'

def setup_inputs():
    _rng = _Rng(jax.random.key(int.from_bytes(__import__("os").urandom(4), "little")))
    _w = lambda a: (lambda t: t.astype(jnp.bfloat16) if jnp.issubdtype(t.dtype, jnp.floating) else t)(jnp.asarray(a))

    def _A_setup():
        B, S, D = (1, 2048, 576)
        return {'x': _w((lambda *s: _rng.normal(s) * 0.05)(B, S, D)), 'wqkv': _w((lambda *s: _rng.normal(s) * 0.05)(D, 3 * D)), 'wo': _w((lambda *s: _rng.normal(s) * 0.05)(D, D))}
    _A_in = _A_setup()

    def _B_setup():
        B, S, D, Dff = (1, 2048, 576, 4608)
        return {'x': _w((lambda *s: _rng.normal(s) * 0.05)(B, S, D)), 'w1': _w((lambda *s: _rng.normal(s) * 0.05)(D, Dff)), 'w2': _w((lambda *s: _rng.normal(s) * 0.05)(Dff, D))}
    _B_in = _B_setup()
    return {'A_x': _A_in['x'], 'A_wqkv': _A_in['wqkv'], 'A_wo': _A_in['wo'], 'B_x': _B_in['x'], 'B_w1': _B_in['w1'], 'B_w2': _B_in['w2'], 'c': _w((lambda *s: _rng.normal(s) * 0.05)(1, 576) * 8.0), 'w_mod': _w((lambda *s: _rng.normal(s) * 0.05)(576, 6 * 576) * 576 ** (-0.5) * 8.0)}

def reference(A_x, A_wqkv, A_wo, B_x, B_w1, B_w2, c, w_mod):

    def _A_ref(x, wqkv, wo):
        B, S, D = x.shape
        H = 32
        Dh = D // H
        W, dil = (8, 2)
        qkv = (lambda x, *d: x.transpose(*d))((x @ wqkv).reshape(B, S, 3, H, Dh), 2, 0, 3, 1, 4)
        q, k, v = (qkv[0], qkv[1], qkv[2])
        scale = Dh ** (-0.5)
        pos = jnp.arange(S)
        off = jnp.arange(W) * dil
        idx = pos[:, None] - off[None, :]
        mask = idx >= 0
        idx_c = jnp.where(mask, idx, 0).reshape(-1)
        kg = k[:, :, idx_c, :].reshape(B, H, S, W, Dh)
        vg = v[:, :, idx_c, :].reshape(B, H, S, W, Dh)
        logits = jnp.einsum('bhsd,bhswd->bhsw', q, kg) * scale
        logits = jnp.where(mask[None, None, :, :], logits, -1000000000.0)
        attn = _softmax(logits, axis=-1)
        o = jnp.einsum('bhsw,bhswd->bhsd', attn, vg)
        return (lambda x, *d: x.transpose(*d))(o, 0, 2, 1, 3).reshape(B, S, D) @ wo

    def _B_ref(x, w1, w2):
        h = jnp.einsum('bsd,df->bsf', x, w1)
        zero = jnp.zeros_like(h)
        h = jnp.maximum(h, zero)
        return jnp.einsum('bsf,fd->bsd', h, w2)
    x = A_x
    mod = (_silu(c) @ w_mod).reshape(c.shape[0], 6, 1, -1)
    sa, ca, ga, sb, cb, gb = (mod[:, 0].copy(), mod[:, 1].copy(), mod[:, 2].copy(), mod[:, 3].copy(), mod[:, 4].copy(), mod[:, 5].copy())
    h = _layernorm(x, axis=-1) * (1 + ca) + sa
    x = x + ga * _A_ref(h, A_wqkv, A_wo)
    h = _layernorm(x, axis=-1) * (1 + cb) + sb
    x = x + gb * _B_ref(h, B_w1, B_w2)
    return x
```

```python
import jax
import jax.numpy as jnp
import numpy as np
from jax import lax
from jax.experimental import pallas as pl
from jax.experimental.pallas import tpu as pltpu

S, D, F = 2048, 576, 4608
DH, WIN = 18, 8
DP = 640
NP = 1792
T = 256
NB = S // T
FC = 1536
SPLIT = 2 * T
EPS = 1e-5
LOG2E = 1.4426950408889634
QSCALE = (DH ** -0.5) * LOG2E
MASKED = -1e9 * LOG2E
NT = (((1,), (1,)), ((), ()))
f32, bf16, u32 = jnp.float32, jnp.bfloat16, jnp.uint32


def _ln_mod(x, scale1p, shift):
    m = jnp.mean(x, axis=0, keepdims=True)
    xc = x - m
    v = jnp.mean(xc * xc, axis=0, keepdims=True)
    r = lax.rsqrt(v + EPS)
    outs = []
    for j in range(x.shape[1] // 128):
        sl = slice(j * 128, (j + 1) * 128)
        outs.append((xc[:, sl] * r[:, sl]) * scale1p + shift)
    return jnp.concatenate(outs, axis=1)


def _pack(v):
    return pltpu.bitcast(v, u32)


def _ld(ref, r0, r1):
    return pltpu.bitcast(ref[r0 // 2:r1 // 2, :], bf16)


def _st_t(ref, r0, h_t):
    hp = jnp.concatenate([h_t, jnp.zeros((DP - D, h_t.shape[1]), h_t.dtype)], axis=0).T
    ref[r0 // 2:(r0 + h_t.shape[1]) // 2, :] = _pack(hp)


def _qkv_row(s, d):
    if d < 16:
        return (0, 512, 1152)[s] + d * 32
    return (1024, 1088, 1664)[s] + (d - 16) * 32


def _kernel(xT_hbm, wqkv_hbm, wo_hbm, w1_hbm, w2T_hbm, c_hbm, wmod_hbm, outT_hbm,
            c_v, xT_v, wqkv_v, wo_v, w1_v, w2T_v, wmod_v, modT, sT, wot, wtu, wpT, woPT,
            q_lo, k_lo, v_lo, q_hi, k_hi, v_hi, o_s, h1_s, h2_s, x2_s, out_s, acc_s,
            sems, osem, fsem):
    def cols(src, dst, c0, c1, i):
        return pltpu.make_async_copy(src.at[:, c0:c1], dst.at[:, c0:c1], sems.at[i])

    cps = {
        "wqkv_a": cols(wqkv_hbm, wqkv_v, 384, 640, 0),
        "wqkv_0": cols(wqkv_hbm, wqkv_v, 0, 384, 12),
        "wqkv_b": cols(wqkv_hbm, wqkv_v, 640, 1152, 1),
        "wqkv_c": cols(wqkv_hbm, wqkv_v, 1152, 1728, 2),
        "wmod_a": cols(wmod_hbm, wmod_v, 0, 1152, 3),
        "x_0": cols(xT_hbm, xT_v, 0, T, 4),
        "c": pltpu.make_async_copy(c_hbm, c_v, sems.at[11]),
        "x_1": cols(xT_hbm, xT_v, T, 2 * T, 10),
        "x_b": cols(xT_hbm, xT_v, 2 * T, S, 5),
        "wmod_b": cols(wmod_hbm, wmod_v, 1152, 6 * D, 6),
        "wo": pltpu.make_async_copy(wo_hbm, wo_v, sems.at[7]),
        "w1": pltpu.make_async_copy(w1_hbm, w1_v, sems.at[8]),
        "w2": pltpu.make_async_copy(w2T_hbm, w2T_v, sems.at[9]),
    }
    for name in ("c", "wmod_a", "wqkv_0", "x_0", "wqkv_a", "x_1", "wqkv_b", "wqkv_c",
                 "x_b", "wmod_b", "wo", "w1", "w2"):
        cps[name].start()

    def wait(*names):
        for name in names:
            cps[name].wait()

    def fence():
        pl.semaphore_signal(fsem.at[0], 1)
        pl.semaphore_wait(fsem.at[0], 1)

    def transpose_wqkv(n0, n1):
        for n in range(n0, n1):
            c0 = n * 128
            cw = min(128, 3 * D - c0)
            for kt in range(5):
                rw = min(128, D - kt * 128)
                blk = wqkv_v[kt * 128:kt * 128 + rw, c0:c0 + cw]
                if rw < 128:
                    blk = jnp.concatenate([blk, jnp.zeros((128 - rw, cw), bf16)], axis=0)
                if cw < 128:
                    blk = jnp.concatenate([blk, jnp.zeros((128, 128 - cw), bf16)], axis=1)
                wtu[kt, c0 // 2:c0 // 2 + 64, :] = _pack(blk.T)

    def gather_wqkv(s):
        for e in range(DH // 2):
            base = s * (D // 2) + e
            for kt in range(5):
                ev = wtu[kt, pl.ds(base, 16, stride=DH), :]
                od = wtu[kt, pl.ds(base + DH // 2, 16, stride=DH), :]
                lo = (ev & np.uint32(0xFFFF)) | (od << 16)
                hi = (ev >> 16) | (od & np.uint32(0xFFFF0000))
                for d, val in ((2 * e, lo), (2 * e + 1, hi)):
                    r = _qkv_row(s, d) // 2
                    wpT[r:r + 16, kt * 128:(kt + 1) * 128] = val

    def prep_wo():
        for kt in range(5):
            cw = min(128, D - kt * 128)
            blk = wo_v[:, kt * 128:kt * 128 + cw].astype(f32)
            if cw < 128:
                blk = jnp.concatenate([blk, jnp.zeros((D, 128 - cw), f32)], axis=1)
            wot[kt, 0:D, :] = blk
        for a in range(5):
            for kt in range(5):
                parts = []
                for d in range(4 * a, 4 * a + 4):
                    if d < DH:
                        parts.append(wot[kt, pl.ds(d, 32, stride=DH), :])
                    else:
                        parts.append(jnp.zeros((32, 128), f32))
                blk = jnp.concatenate(parts, axis=0).T.astype(bf16)
                rw = min(128, D - kt * 128)
                woPT[kt * 64:kt * 64 + rw // 2, a * 128:(a + 1) * 128] = _pack(blk[:rw])

    def silu_c():
        cv = c_v[...].astype(f32)
        return (cv * jax.nn.sigmoid(cv)).astype(bf16)

    def store_mod(n, row):
        if (n * 128 < 2 * D and (n + 1) * 128 > D) or (n * 128 < 5 * D and (n + 1) * 128 > 4 * D):
            col = lax.broadcasted_iota(jnp.int32, (1, 128), 1) + n * 128
            is_scale = ((col >= D) & (col < 2 * D)) | ((col >= 4 * D) & (col < 5 * D))
            row = row + jnp.where(is_scale, 1.0, 0.0)
        modT[n * 128:(n + 1) * 128, :] = jnp.broadcast_to(row, (128, 128)).T

    def mod_first():
        mod = jnp.dot(jnp.broadcast_to(silu_c(), (16, D)), wmod_v[:, 0:1152],
                      preferred_element_type=f32)
        for n in range(9):
            store_mod(n, mod[0:1, n * 128:(n + 1) * 128])
        sv = jnp.concatenate([silu_c().astype(f32), jnp.zeros((1, DP - D), f32)], axis=1)
        for kt in range(5):
            rw = min(128, D - kt * 128)
            sT[kt * 128:kt * 128 + rw, :] = jnp.broadcast_to(
                sv[:, kt * 128:(kt + 1) * 128], (128, 128)).T[:rw]
        for a in range(5):
            k_lo[a, 0:16, :] = jnp.zeros((16, 128), f32)
            v_lo[a, 0:16, :] = jnp.zeros((16, 128), f32)

    def mod_rest():
        for g0 in range(9, 27, 3):
            accs = [None] * 3
            for r in range(0, D, 16):
                sv = sT[r:r + 16, :]
                for u in range(3):
                    n = g0 + u
                    t = sv * wmod_v[r:r + 16, n * 128:(n + 1) * 128].astype(f32)
                    t = t[0:8] + t[8:16]
                    accs[u] = t if accs[u] is None else accs[u] + t
            for u in range(3):
                store_mod(g0 + u, jnp.sum(accs[u], axis=0, keepdims=True))

    def modv(j):
        return modT[j * D:(j + 1) * D, :]

    class Blocks:
        def __init__(self, i0, n):
            self.static = isinstance(i0, int)
            t0 = i0 * T if self.static else pl.multiple_of(i0 * T, T)
            t2 = i0 * (T // 2) if self.static else pl.multiple_of(i0 * (T // 2), T // 2)
            self.t0 = t0
            self.xT = xT_v.at[:, pl.ds(t0, n * T)]
            self.x2 = x2_s.at[:, pl.ds(t0, n * T)]
            self.out = out_s.at[:, pl.ds(t0, n * T)]
            self.out_hbm = outT_hbm.at[:, pl.ds(t0, n * T)]
            self.h1 = h1_s.at[pl.ds(t2, n * T // 2), :]
            self.h2 = h2_s.at[pl.ds(t2, n * T // 2), :]
            self.o = o_s.at[pl.ds(t0, n * T), :]

    def qkv_views(r0, n, low):
        if low:
            return (q_lo.at[:, pl.ds(r0, n), :], k_lo.at[:, pl.ds(r0, n + 16), :],
                    v_lo.at[:, pl.ds(r0, n + 16), :])
        r1 = r0 - SPLIT
        if not isinstance(r1, int):
            r1 = pl.multiple_of(r1, T)
        return (q_hi.at[:, pl.ds(r1, n), :], k_hi.at[:, pl.ds(r1, n + 16), :],
                v_hi.at[:, pl.ds(r1, n + 16), :])

    def ln1(bl, j):
        x = bl.xT[:, j * T:(j + 1) * T].astype(f32)
        _st_t(bl.h1, j * T, _ln_mod(x, modv(1), modv(0)).astype(bf16))

    def qkv(bl, j, part="qkv"):
        r0 = j * T
        low = bl.t0 + r0 < SPLIT
        q, k, v = qkv_views(bl.t0 + r0, T, low)
        dup = bl.t0 + r0 + T == SPLIT
        n0, n1 = {"qkv": (0, NP), "q": (0, 512), "k": (512, 1152), "v": (1152, NP)}[part]
        y = lax.dot_general(_ld(bl.h1, r0, r0 + T), _ld(wpT, n0, n1), NT,
                            preferred_element_type=f32)

        def tile(n):
            return y[:, n * 128 - n0:(n + 1) * 128 - n0]

        def put(dst, dst_hi, a, val):
            dst[a, 16:16 + T, :] = val
            if dup:
                dst_hi[a, 0:16, :] = val[T - 16:T, :]

        if "q" in part:
            for a in range(4):
                q[a] = tile(a) * QSCALE
        if "k" in part:
            for a in range(4):
                put(k, k_hi, a, tile(4 + a))
            t8 = tile(8)
            lane = lax.broadcasted_iota(jnp.int32, (T, 128), 1)
            q[4] = jnp.where(lane < 64, t8 * QSCALE, 0.0)
            put(k, k_hi, 4, pltpu.roll(t8, 64, 1))
        if "v" in part:
            for a in range(5):
                put(v, v_hi, a, tile(9 + a))

    def attention(r0, nrows, rg, o):
        static = isinstance(r0, int)
        if not static:
            r0 = pl.multiple_of(r0, 8)
        q, k, v = qkv_views(r0, nrows, static and r0 < SPLIT)
        for base in range(0, nrows, rg):
            row = lax.broadcasted_iota(jnp.int32, (rg, 128), 0)
            qs = [q[a, base:base + rg, :] for a in range(5)]
            ls = []
            for w in range(WIN):
                kb = base + 16 - 2 * w
                acc = None
                for a in range(5):
                    t = qs[a] * k[a, kb:kb + rg, :]
                    acc = t if acc is None else acc + t
                acc = acc + pltpu.roll(acc, 64, 1)
                acc = acc + pltpu.roll(acc, 32, 1)
                if static and r0 + base < 2 * w:
                    acc = jnp.where(row + (r0 + base) >= 2 * w, acc, MASKED)
                ls.append(acc)
            m = ls[0]
            for w in range(1, WIN):
                m = jnp.maximum(m, ls[w])
            p = [jnp.exp2(lg - m) for lg in ls]
            den = p[0]
            for w in range(1, WIN):
                den = den + p[w]
            rinv = 1.0 / den
            for a in range(5):
                oo = None
                for w in range(WIN):
                    vb = base + 16 - 2 * w
                    t = p[w] * v[a, vb:vb + rg, :]
                    oo = t if oo is None else oo + t
                o[base:base + rg, a * 128:(a + 1) * 128] = (oo * rinv).astype(bf16)

    def attn_block(bl, j, rg, g0=0, g1=None):
        g1 = T // rg if g1 is None else g1
        lo, n = j * T + g0 * rg, (g1 - g0) * rg
        attention(bl.t0 + lo, n, rg, bl.o.at[lo:lo + n, :])

    def out_proj(bl, j):
        y = lax.dot_general(_ld(woPT, 0, D), bl.o[j * T:(j + 1) * T, :], NT,
                            preferred_element_type=f32)
        ga = modv(2)
        x = bl.xT[:, j * T:(j + 1) * T].astype(f32)
        bl.x2[:, j * T:(j + 1) * T] = jnp.concatenate(
            [x[:, u * 128:(u + 1) * 128] + ga * y[:, u * 128:(u + 1) * 128]
             for u in range(T // 128)], axis=1)

    def ln2(bl, j):
        x2 = bl.x2[:, j * T:(j + 1) * T]
        _st_t(bl.h2, j * T, _ln_mod(x2, modv(4), modv(3)).astype(bf16))

    def ffn_up(bl, j, c):
        h2 = _ld(bl.h2, j * T, (j + 1) * T)[:, :D]
        a = jnp.dot(h2, w1_v[:, c * FC:(c + 1) * FC], preferred_element_type=f32)
        return jnp.maximum(a, 0.0).astype(bf16)

    def ffn_down(act, c, acc=None):
        r = lax.dot_general(w2T_v[:, c * FC:(c + 1) * FC], act, NT, preferred_element_type=f32)
        return r if acc is None else acc + r

    def emit(bl, c0, n, acc):
        gb = modv(5)
        x2 = bl.x2[:, c0:c0 + n]
        res = jnp.concatenate(
            [x2[:, u * 128:(u + 1) * 128] + gb * acc[:, u * 128:(u + 1) * 128]
             for u in range(n // 128)], axis=1)
        bl.out[:, c0:c0 + n] = res.astype(bf16)
        pltpu.make_async_copy(bl.out.at[:, c0:c0 + n], bl.out_hbm.at[:, c0:c0 + n],
                              osem.at[0]).start()

    g = Blocks(0, NB)
    wait("c", "wmod_a")
    mod_first()
    wait("wqkv_0")
    transpose_wqkv(0, 3)
    wait("x_0")
    ln1(g, 0)
    wait("wqkv_a")
    transpose_wqkv(3, 5)
    gather_wqkv(0)
    wpT[864:896, :] = jnp.zeros((32, DP), u32)
    wait("x_1")
    qkv(g, 0, "q")
    ln1(g, 1)
    wait("wqkv_b")
    qkv(g, 1, "q")
    transpose_wqkv(5, 9)
    gather_wqkv(1)
    wait("wqkv_c")
    qkv(g, 0, "k")
    transpose_wqkv(9, 14)
    gather_wqkv(2)
    qkv(g, 1, "k")
    qkv(g, 0, "v")
    wait("x_b")
    attention(0, 128, 8, o_s.at[pl.ds(0, 128), :])
    ln1(g, 2)
    qkv(g, 1, "v")
    ln1(g, 3)
    qkv(g, 2)
    ln1(g, 4)
    qkv(g, 3)
    fence()
    attention(128, 128, 8, o_s.at[pl.ds(128, 128), :])
    ln1(g, 5)
    qkv(g, 4)
    ln1(g, 6)
    qkv(g, 5)
    wait("wmod_b", "wo")
    ln1(g, 7)
    qkv(g, 6)
    mod_rest()
    prep_wo()
    out_proj(g, 0)
    qkv(g, 7)
    ln2(g, 0)
    wait("w1", "w2")

    b = Blocks(0, 3)
    acc = ffn_down(ffn_up(b, 0, 0), 0)
    acc = ffn_down(ffn_up(b, 0, 1), 1, acc)
    attn_block(b, 1, 16)
    attn_block(b, 2, 8, 0, 16)
    fence()
    out_proj(b, 1)
    acc_s[...] = ffn_down(ffn_up(b, 0, 2), 2, acc)
    attn_block(b, 2, 8, 16, 32)
    ln2(b, 1)

    def ffn_step(bl, attn, proj, order):
        act = ffn_up(bl, 1, 0)
        emit(bl, 0, T, acc_s[...])
        if proj and order == 0:
            out_proj(bl, 2)
        acc = ffn_down(act, 0)
        if proj and order == 1:
            out_proj(bl, 2)
        acc = ffn_down(ffn_up(bl, 1, 1), 1, acc)
        act = ffn_up(bl, 1, 2)
        if not proj:
            return act, acc
        acc_s[...] = ffn_down(act, 2, acc)
        if attn:
            attn_block(bl, 3, 8)
        ln2(bl, 2)

    def body(i, carry):
        ffn_step(Blocks(i - 1, 4), True, True, 0)
        return carry

    lax.fori_loop(1, NB - 2, body, 0)
    ffn_step(Blocks(NB - 3, 3), False, True, 1)
    last = Blocks(NB - 2, 2)
    act, acc = ffn_step(last, False, False, 0)
    for u in range(T // 128):
        sl = slice(u * 128, (u + 1) * 128)
        emit(last, T + u * 128, 128, ffn_down(act[sl], 2, acc[:, sl]))
    pltpu.make_async_copy(out_s, outT_hbm, osem.at[0]).wait()


def _scratch_shapes():
    return [
        pltpu.VMEM((1, D), bf16),
        pltpu.VMEM((D, S), bf16),
        pltpu.VMEM((D, 3 * D), bf16),
        pltpu.VMEM((D, D), bf16),
        pltpu.VMEM((D, F), bf16),
        pltpu.VMEM((D, F), bf16),
        pltpu.VMEM((D, 6 * D), bf16),
        pltpu.VMEM((6 * D, 128), f32),
        pltpu.VMEM((D, 128), f32),
        pltpu.VMEM((5, D, 128), f32),
        pltpu.VMEM((5, NP // 2, 128), u32),
        pltpu.VMEM((NP // 2, DP), u32),
        pltpu.VMEM((D // 2, DP), u32),
        pltpu.VMEM((5, SPLIT, 128), f32),
        pltpu.VMEM((5, SPLIT + 16, 128), f32),
        pltpu.VMEM((5, SPLIT + 16, 128), f32),
        pltpu.VMEM((5, S - SPLIT, 128), f32),
        pltpu.VMEM((5, S - SPLIT + 16, 128), f32),
        pltpu.VMEM((5, S - SPLIT + 16, 128), f32),
        pltpu.VMEM((S, DP), bf16),
        pltpu.VMEM((S // 2, DP), u32),
        pltpu.VMEM((S // 2, DP), u32),
        pltpu.VMEM((D, S), f32),
        pltpu.VMEM((D, S), bf16),
        pltpu.VMEM((D, T), f32),
        pltpu.SemaphoreType.DMA((13,)),
        pltpu.SemaphoreType.DMA((1,)),
        pltpu.SemaphoreType.REGULAR((1,)),
    ]


def run(A_x, A_wqkv, A_wo, B_x, B_w1, B_w2, c, w_mod):
    del B_x
    hbm = pl.BlockSpec(memory_space=pl.ANY)
    outT = pl.pallas_call(
        _kernel,
        out_shape=jax.ShapeDtypeStruct((D, S), bf16),
        in_specs=[hbm] * 7,
        out_specs=hbm,
        scratch_shapes=_scratch_shapes(),
        compiler_params=pltpu.CompilerParams(vmem_limit_bytes=100 * 1024 * 1024),
        name="adaln_fused",
    )(A_x.reshape(S, D).T, A_wqkv, A_wo, B_w1, B_w2.T, c, w_mod)
    return outT.T.reshape(1, S, D)


@jax.jit
def pallas_adaLN_cond__sliding_local_dilated__dense_activation_relu__prompt_kernel(
    A_x: jax.Array,
    A_wqkv: jax.Array,
    A_wo: jax.Array,
    B_x: jax.Array,
    B_w1: jax.Array,
    B_w2: jax.Array,
    c: jax.Array,
    w_mod: jax.Array,
):
    return run(A_x, A_wqkv, A_wo, B_x, B_w1, B_w2, c, w_mod)
```
